```python
import os as _os
_os.environ.setdefault("JAX_PLATFORMS", "cpu")
import jax
import jax.numpy as jnp

def _softmax(x, axis=-1):
    return jax.nn.softmax(x, axis=axis)
def _gelu(x):
    return jax.nn.gelu(x, approximate=True)
def _silu(x):
    return jax.nn.silu(x)
def _sigmoid(x):
    return jax.nn.sigmoid(x)
def _layernorm(x, axis=-1, eps=1e-5):
    m = jnp.mean(x, axis=axis, keepdims=True)
    v = jnp.var(x, axis=axis, keepdims=True)
    return (x - m) / jnp.sqrt(v + eps)
def _scatter_add(tgt, idx, src, axis=0):
    return tgt.at[idx].add(src)
def _segment_sum(src, seg, n):
    return jax.ops.segment_sum(src, seg, n)
class _Rng:
    def __init__(self, key):
        self._k = key
    def _next(self):
        self._k, sub = jax.random.split(self._k)
        return sub
    def normal(self, shape):
        return jax.random.normal(self._next(), shape, dtype=jnp.bfloat16)
    def randint(self, lo, hi, shape):
        return jax.random.randint(self._next(), shape, lo, hi, dtype=jnp.int32)
    def uniform(self, shape, lo=0.0, hi=1.0):
        return jax.random.uniform(self._next(), shape, jnp.bfloat16, lo, hi)
    def permutation(self, n):
        return jax.random.permutation(self._next(), n)


kernel_name = 'concat_heads__gqa_block_cached__sliding_block_cached__decode'

def setup_inputs():
    _rng = _Rng(jax.random.key(int.from_bytes(__import__("os").urandom(4), "little")))
    _w = (lambda a: (lambda t: t.astype(jnp.bfloat16) if jnp.issubdtype(t.dtype, jnp.floating) else t)(jnp.asarray(a)))
    def _A_setup():
        B, Sq, D = 2, 1, 448
        Hq, Hkv, Sk, Dh = 16, 8, 8192, 256
        assert Hq % Hkv == 0, (Hq, Hkv)
        return {
            "x": _w((lambda *s: _rng.normal(s) * 0.8)(B, Sq, D)),
            "k_cache": _w((lambda *s: _rng.normal(s) * 0.8)(B, Hkv, Sk, Dh)),
            "v_cache": _w((lambda *s: _rng.normal(s) * 0.05)(B, Hkv, Sk, Dh)),
            "wq": _w((lambda *s: _rng.normal(s) * 0.8)(D, Hq * Dh) * (D ** -0.5)),
            "wo": _w((lambda *s: _rng.normal(s) * 0.05)(Hq * Dh, D) * ((Hq * Dh) ** -0.5)),
        }
    _A_in = _A_setup()

    def _B_setup():
        B, Sq, D = 2, 1, 448
        Hq, Hkv, Sk, Dh = 16, 8, 8192, 256
        assert Hq % Hkv == 0, (Hq, Hkv)
        return {
            "x": _w((lambda *s: _rng.normal(s) * 0.8)(B, Sq, D)),
            "k_cache": _w((lambda *s: _rng.normal(s) * 0.8)(B, Hkv, Sk, Dh)),
            "v_cache": _w((lambda *s: _rng.normal(s) * 0.05)(B, Hkv, Sk, Dh)),
            "wq": _w((lambda *s: _rng.normal(s) * 0.8)(D, Hq * Dh) * (D ** -0.5)),
            "wo": _w((lambda *s: _rng.normal(s) * 0.05)(Hq * Dh, D) * ((Hq * Dh) ** -0.5)),
        }
    _B_in = _B_setup()

    return {
        "A_x": _A_in["x"],
        "A_k_cache": _A_in["k_cache"],
        "A_v_cache": _A_in["v_cache"],
        "A_wq": _A_in["wq"],
        "A_wo": _A_in["wo"],
        "B_x": _B_in["x"],
        "B_k_cache": _B_in["k_cache"],
        "B_v_cache": _B_in["v_cache"],
        "B_wq": _B_in["wq"],
        "B_wo": _B_in["wo"],
    }

def reference(A_x, A_k_cache, A_v_cache, A_wq, A_wo, B_x, B_k_cache, B_v_cache, B_wq, B_wo):
    def _A_ref(x, k_cache, v_cache, wq, wo):
        B, Sq, D = x.shape
        Hq, Dh = 16, 256
        Hkv = k_cache.shape[1]
        rep = Hq // Hkv
        q = (lambda x, *d: x.transpose(*d))((x @ wq).reshape(B, Sq, Hq, Dh), 0, 2, 1, 3)
        k = jnp.repeat(k_cache, rep, axis=1)
        v = jnp.repeat(v_cache, rep, axis=1)
        scores = jnp.einsum("bhqd,bhkd->bhqk", q, k) * (Dh ** -0.5)
        p = _softmax(scores, axis=-1)
        o = jnp.einsum("bhqk,bhkd->bhqd", p, v)
        return (lambda x, *d: x.transpose(*d))(o, 0, 2, 1, 3).reshape(B, Sq, Hq * Dh) @ wo

    def _B_ref(x, k_cache, v_cache, wq, wo):
        B, Sq, D = x.shape
        Hq, Dh = 16, 256
        Hkv, Sk = k_cache.shape[1], k_cache.shape[2]
        W = min(4096, max(256, Sk // 4))
        rep = Hq // Hkv
        q = (lambda x, *d: x.transpose(*d))((x @ wq).reshape(B, Sq, Hq, Dh), 0, 2, 1, 3)
        k = jnp.repeat(k_cache[:, :, Sk - W:, :], rep, axis=1)
        v = jnp.repeat(v_cache[:, :, Sk - W:, :], rep, axis=1)
        scores = jnp.einsum("bhqd,bhkd->bhqk", q, k) * (Dh ** -0.5)
        p = _softmax(scores, axis=-1)
        o = jnp.einsum("bhqk,bhkd->bhqd", p, v)
        return (lambda x, *d: x.transpose(*d))(o, 0, 2, 1, 3).reshape(B, Sq, Hq * Dh) @ wo

    a = _A_ref(A_x, A_k_cache, A_v_cache, A_wq, A_wo)
    b = _B_ref(B_x, B_k_cache, B_v_cache, B_wq, B_wo)
    return jnp.concatenate([a, b], axis=-1)
```

```python
import functools
import jax
import jax.numpy as jnp
from jax import lax
import jax.experimental.pallas as pl
import jax.experimental.pallas.tpu as pltpu

HQ, DH = 16, 256
NT = (((1,), (1,)), ((), ()))
NN = (((1,), (0,)), ((), ()))


def build(R=1024, SUB=64, NBUF=4, LOOK=2, nobc=False, compute=True):
    assert LOOK < NBUF

    def kernel(ax, ak, av, awq, awo, bx, bk, bv, bwq, bwo, o_ref,
               xbuf, wqbuf, wobuf, kbuf, vbuf, qs, os_, m_s, l_s, acc_s, sem_x, sem_w, sem_kv,
               *, nb, hkv, sk, win, d):
        ca = sk // R
        cb = win // R
        na = nb * hkv * ca
        ntot = na + nb * hkv * cb
        gw = 2 * DH
        wrows = SUB * DH // gw
        nw = hkv

        def start_w(a_src, b_src, dst, which, g):
            for j in range(d // wrows):
                for p, src in enumerate((a_src, b_src)):
                    pltpu.make_async_copy(
                        src.at[pl.ds(j * wrows, wrows), pl.ds(g * gw, gw)],
                        dst.at[g, p, pl.ds(j * wrows, wrows), :],
                        sem_w.at[which, g]).start(priority=p)

        def wait_w(dst, which, g):
            pltpu.make_async_copy(dst.at[g], dst.at[g], sem_w.at[which, g]).wait()

        def start_kv(k_src, v_src, base, slot):
            for j in range(R // SUB):
                pltpu.make_async_copy(k_src.at[pl.ds(base + j * SUB, SUB)],
                                      kbuf.at[slot, pl.ds(j * SUB, SUB)], sem_kv.at[0, slot]).start(priority=0)
                pltpu.make_async_copy(v_src.at[pl.ds(base + j * SUB, SUB)],
                                      vbuf.at[slot, pl.ds(j * SUB, SUB)], sem_kv.at[1, slot]).start(priority=1)

        def base_a(t):
            return t * R

        def base_b(t):
            u = t - na
            return (u // cb) * sk + (sk - win) + (u % cb) * R

        def start_static(g):
            if g < nw:
                start_w(awq, bwq, wqbuf, 0, g)
            elif g < nw + ntot:
                t = g - nw
                if t < na:
                    start_kv(ak, av, base_a(t), t % NBUF)
                else:
                    start_kv(bk, bv, base_b(t), t % NBUF)
            elif g < 2 * nw + ntot:
                start_w(awo, bwo, wobuf, 1, g - nw - ntot)

        for g in range(LOOK):
            start_static(g)
            if g == 0:
                xa = pltpu.make_async_copy(ax, xbuf.at[0], sem_x.at[0])
                xb = pltpu.make_async_copy(bx, xbuf.at[1], sem_x.at[1])
                xa.start(priority=0)
                xb.start(priority=1)

        row8 = lax.broadcasted_iota(jnp.int32, (8, DH), 0)
        os_[...] = jnp.zeros(os_.shape, os_.dtype)
        xa.wait()
        xb.wait()
        rowx = lax.broadcasted_iota(jnp.int32, (16, d), 0)
        x16 = []
        for p in range(2):
            xv = xbuf[p].astype(jnp.float32)
            x16.append(jnp.where(rowx % 2 == 0, xv[0:1, :], xv[1:2, :]).astype(jnp.bfloat16))

        row16 = lax.broadcasted_iota(jnp.int32, (16, DH), 0)
        for g in range(nw):
            wait_w(wqbuf, 0, g)
            start_static(g + LOOK)
            for p in range(2):
                y = lax.dot_general(x16[p], wqbuf[g, p], NN, preferred_element_type=jnp.float32)
                qs[p * hkv + g] = jnp.where(row16 < 2, y[:, :DH], y[:, DH:]).astype(jnp.bfloat16)

        def step(t, is_b, issue):
            slot = t % NBUF
            pltpu.make_async_copy(kbuf.at[slot], kbuf.at[slot], sem_kv.at[0, slot]).wait()
            pltpu.make_async_copy(vbuf.at[slot], vbuf.at[slot], sem_kv.at[1, slot]).wait()
            issue()
            if not compute:
                return
            if is_b:
                u = t - na
                bh, c, nc, p = u // cb, u % cb, cb, 1
            else:
                bh, c, nc, p = t // ca, t % ca, ca, 0
            b = bh // hkv
            h = bh % hkv

            @pl.when(c == 0)
            def _():
                m_s[...] = jnp.full(m_s.shape, -jnp.inf, jnp.float32)
                l_s[...] = jnp.zeros(l_s.shape, jnp.float32)
                acc_s[...] = jnp.zeros(acc_s.shape, jnp.float32)

            q = qs[p * hkv + h]
            s = lax.dot_general(q, kbuf[slot], NT, preferred_element_type=jnp.float32)[0:8] * (DH ** -0.5)
            m_old = m_s[...]
            m_new = jnp.maximum(m_old, jnp.max(s, axis=1, keepdims=True))
            alpha = jnp.exp(m_old - m_new)
            pr = jnp.exp(s - m_new[:, 0:1])
            l_new = alpha * l_s[...] + jnp.sum(pr, axis=1, keepdims=True)
            pv = lax.dot_general(pr.astype(jnp.bfloat16), vbuf[slot], NN, preferred_element_type=jnp.float32)
            acc = jnp.concatenate([alpha, alpha], axis=1) * acc_s[...] + pv
            m_s[...] = m_new
            l_s[...] = l_new
            acc_s[...] = acc

            @pl.when(c == nc - 1)
            def _():
                o = acc / jnp.concatenate([l_new, l_new], axis=1)
                j = p * HQ + 2 * h
                os_[j] = jnp.where(row8 == b, o, os_[j])
                os_[j + 1] = jnp.where(row8 == b, pltpu.roll(o, 6, 0), os_[j + 1])

        def body_a(t, c):
            def issue():
                t2 = t + LOOK
                start_kv(ak, av, pl.multiple_of(base_a(t2), R), t2 % NBUF)
            step(t, False, issue)
            return c

        def body_b(t, c):
            def issue():
                t2 = t + LOOK
                start_kv(bk, bv, pl.multiple_of(base_b(t2), R), t2 % NBUF)
            step(t, True, issue)
            return c

        lax.fori_loop(0, na - LOOK, body_a, 0)
        for t in range(na - LOOK, na):
            step(t, False, lambda: start_static(nw + t + LOOK))
        lax.fori_loop(na, ntot - LOOK, body_b, 0)
        for t in range(ntot - LOOK, ntot):
            step(t, True, lambda: start_static(nw + t + LOOK))

        outs = [jnp.zeros((8, d), jnp.float32), jnp.zeros((8, d), jnp.float32)]
        for g in range(nw):
            wait_w(wobuf, 1, g)
            start_static(nw + ntot + g + LOOK)
            for p in range(2):
                j = p * HQ + 2 * g
                o2 = jnp.concatenate([os_[j], os_[j + 1]], axis=1).astype(jnp.bfloat16)
                outs[p] = outs[p] + lax.dot_general(o2, wobuf[g, p], NT, preferred_element_type=jnp.float32)
        res = jnp.concatenate([outs[0][0:2], outs[1][0:2]], axis=1)
        o_ref[...] = res.astype(o_ref.dtype)

    @jax.jit
    def f(A_x, A_k_cache, A_v_cache, A_wq, A_wo, B_x, B_k_cache, B_v_cache, B_wq, B_wo):
        nb, sq, d = A_x.shape
        _, hkv, sk, dh = A_k_cache.shape
        win = min(4096, max(256, sk // 4))
        n = nb * hkv * sk
        kern = functools.partial(kernel, nb=nb, hkv=hkv, sk=sk, win=win, d=d)
        out = pl.pallas_call(
            kern,
            in_specs=[pl.BlockSpec(memory_space=pl.ANY)] * 10,
            out_specs=pl.BlockSpec(memory_space=pltpu.VMEM),
            out_shape=jax.ShapeDtypeStruct((nb, 2 * d), A_x.dtype),
            scratch_shapes=[
                pltpu.VMEM((2, nb, d), jnp.bfloat16),
                pltpu.VMEM((hkv, 2, d, 2 * DH), jnp.bfloat16),
                pltpu.VMEM((hkv, 2, d, 2 * DH), jnp.bfloat16),
                pltpu.VMEM((NBUF, R, DH), jnp.bfloat16),
                pltpu.VMEM((NBUF, R, DH), jnp.bfloat16),
                pltpu.VMEM((2 * hkv, 16, DH), jnp.bfloat16),
                pltpu.VMEM((2 * HQ, 8, DH), jnp.float32),
                pltpu.VMEM((8, 128), jnp.float32),
                pltpu.VMEM((8, 128), jnp.float32),
                pltpu.VMEM((8, DH), jnp.float32),
                pltpu.SemaphoreType.DMA((2,)),
                pltpu.SemaphoreType.DMA((2, hkv)),
                pltpu.SemaphoreType.DMA((2, NBUF)),
            ],
            compiler_params=pltpu.CompilerParams(vmem_limit_bytes=64 * 1024 * 1024, disable_bounds_checks=nobc),
        )(A_x.reshape(nb, d), A_k_cache.reshape(n, dh), A_v_cache.reshape(n, dh), A_wq, A_wo.T,
          B_x.reshape(nb, d), B_k_cache.reshape(n, dh), B_v_cache.reshape(n, dh), B_wq, B_wo.T)
        return out.reshape(nb, sq, 2 * d)
    return f


pallas_concat_heads__gqa_block_cached__sliding_block_cached__decode_kernel = build(LOOK=4, NBUF=5)
```

```python
import functools
import jax
import jax.numpy as jnp
from jax import lax
import jax.experimental.pallas as pl
import jax.experimental.pallas.tpu as pltpu

HQ, DH = 16, 256
NT = (((1,), (1,)), ((), ()))
NN = (((1,), (0,)), ((), ()))
R = 1024
S = 4
SUB = 64
GR = 64
WC = 2048


def pick(i, table, default):
    out = default
    for k, v in table:
        out = jnp.where(i == k, v, out)
    return out


def build(NBUF=3, LOOK=3, nobc=True, nosc=True, compute=True, phases=(3, 2, 1), nlast=4, SQ=4, olook=3):

    def kernel(ax, ak, av, awq, awo, bx, bk, bv, bwq, bwo, o_ref,
               xbuf, xs, wqbuf, wobuf, kvbuf, ys, qs, os_, res, m_s, l_s, acc_s, sem_x, sem_q, sem_o, sem_kv,
               *, nb, hkv, sk, win, d):
        hd = HQ * DH
        nw = d // GR
        ca, cb = sk // R, win // R
        na = nb * hkv * ca
        nkv = na + nb * hkv * cb
        total = 2 * nw + nkv
        lag = S - 1 + LOOK
        ppg = (GR // 8) * (hd // WC)
        lc = hd // nlast
        starts = [sum(phases[:i]) for i in range(len(phases))]
        nq = S
        qper = pl.cdiv(2 * nw, nq)
        q0 = nw + lag - nq
        assert q0 > nw and lag <= (NBUF - 1) * S and sum(phases) == nw - 1 and S % cb == 0 and ca % S == 0

        def start_w(srcs, dst_of, j, ns, length, base, sem):
            def body(i, c):
                idx = j * ppg + i
                piece = base + lax.rem(idx, ns) * length + lax.div(idx, ns)
                row = pl.multiple_of(lax.shift_right_logical(piece, 1) * 8, 8)
                col = pl.multiple_of((piece & 1) * WC, WC)
                for p in range(2):
                    pltpu.make_async_copy(srcs[p].at[pl.ds(row, 8), pl.ds(col, WC)],
                                          dst_of(p, row, col), sem).start(priority=p)
                return c
            lax.fori_loop(0, ppg, body, 0)

        def wo_row(p, row):
            blk = lax.shift_right_logical(row, 6) if not isinstance(row, int) else row // GR
            return blk * (2 * GR) + (p ^ (blk & 1)) * GR + (row & (GR - 1))

        def start_kv(srcs, bases, j, slot):
            per = R // S
            for o in range(0, per, SUB):
                for s in range(S):
                    for w in range(2):
                        pltpu.make_async_copy(
                            srcs[w].at[pl.ds(pl.multiple_of(bases[s] + j * per + o, SUB), SUB)],
                            kvbuf.at[slot, w, s, pl.ds(pl.multiple_of(j * per + o, SUB), SUB)],
                            sem_kv.at[slot]).start(priority=w)

        def issue(g):
            t = g - nw
            i = lax.div(t, S)

            @pl.when((g >= 0) & (t < 0))
            def _():
                start_w((awq, bwq), lambda p, row, col: wqbuf.at[p, pl.ds(row, 8), pl.ds(col, WC)],
                        g, SQ, nw * ppg // SQ, 0, sem_q)

            @pl.when((t >= 0) & (t < na))
            def _():
                start_kv((ak, av), [(i * S + s) * R for s in range(S)], lax.rem(t, S), lax.rem(i, NBUF))

            @pl.when((t >= na) & (t < nkv))
            def _():
                h0 = (i - na // S) * (S // cb)
                start_kv((bk, bv), [(h0 + s // cb) * sk + (sk - win) + (s % cb) * R for s in range(S)],
                         lax.rem(t, S), lax.rem(i, NBUF))

            @pl.when((t >= nkv) & (g < total - 1))
            def _():
                j = t - nkv
                ph, j0, ns = 0, 0, phases[0]
                for k in range(1, len(phases)):
                    ph = jnp.where(j >= starts[k], k, ph)
                    j0 = jnp.where(j >= starts[k], starts[k], j0)
                    ns = jnp.where(j >= starts[k], phases[k], ns)
                start_w((awo, bwo),
                        lambda p, row, col: wobuf.at[pl.ds(pl.multiple_of(wo_row(p, row), 8), 8), pl.ds(col, WC)],
                        j - j0, ns, ppg, j0 * ppg, sem_o.at[ph])

            @pl.when(g == total - 1)
            def _():
                for k in range(nlast):
                    for c0 in range(k * lc, (k + 1) * lc, min(lc, WC)):
                        for row in range(d - GR, d, 8):
                            for p, src in enumerate((awo, bwo)):
                                cols = pl.ds(c0, min(lc, WC))
                                pltpu.make_async_copy(src.at[pl.ds(row, 8), cols],
                                                      wobuf.at[pl.ds(wo_row(p, row), 8), cols],
                                                      sem_o.at[len(phases) + k]).start(priority=p)

        pltpu.make_async_copy(ax, xbuf.at[0], sem_x).start(priority=0)
        pltpu.make_async_copy(bx, xbuf.at[1], sem_x).start(priority=1)

        def prep():
            pltpu.make_async_copy(xbuf, xbuf, sem_x).wait()
            rowx = lax.broadcasted_iota(jnp.int32, (8, d), 0)
            for p in range(2):
                xv = xbuf[p].astype(jnp.float32)
                x8 = jnp.where(rowx % 2 == 0, xv[0:1, :], xv[1:2, :])
                for g in range(nw):
                    xs[g, p] = x8[:, g * GR:(g + 1) * GR]
            ys[...] = jnp.zeros(ys.shape, ys.dtype)
            os_[...] = jnp.zeros(os_.shape, os_.dtype)

        def q_step(k):
            def body(u, c):
                g, p = lax.shift_right_logical(u, 1), u & 1
                w = wqbuf[p, pl.ds(pl.multiple_of(g * GR, GR), GR), :]
                ys[p] = ys[p] + lax.dot_general(xs[g, p].astype(jnp.bfloat16), w, NN,
                                                preferred_element_type=jnp.float32)
                return c
            lax.fori_loop(k * qper, jnp.minimum((k + 1) * qper, 2 * nw), body, 0)

            @pl.when(k == nq - 1)
            def _():
                row8 = lax.broadcasted_iota(jnp.int32, (8, DH), 0)

                def body2(p, c):
                    for h in range(hkv):
                        qs[p * hkv + h] = jnp.where(row8 < 4, ys[p, :, 2 * h * DH:(2 * h + 1) * DH],
                                                    ys[p, :, (2 * h + 1) * DH:(2 * h + 2) * DH])
                    return c
                lax.fori_loop(0, 2, body2, 0)

        def kv_step(t):
            is_b = t >= na
            u = t - na
            p = jnp.where(is_b, 1, 0)
            bh = jnp.where(is_b, lax.div(u, cb), lax.div(t, ca))
            c = jnp.where(is_b, lax.rem(u, cb), lax.rem(t, ca))
            last = jnp.where(is_b, cb - 1, ca - 1)
            b = lax.div(bh, hkv)
            h = lax.rem(bh, hkv)
            slot = lax.rem(lax.div(t, S), NBUF)
            part = lax.rem(t, S)

            @pl.when(c == 0)
            def _():
                m_s[...] = jnp.full(m_s.shape, -jnp.inf, jnp.float32)
                l_s[...] = jnp.zeros(l_s.shape, jnp.float32)
                acc_s[...] = jnp.zeros(acc_s.shape, jnp.float32)

            q = qs[p * hkv + h].astype(jnp.bfloat16)
            s = lax.dot_general(q, kvbuf[slot, 0, part], NT, preferred_element_type=jnp.float32) * (DH ** -0.5)
            m_old = m_s[...]
            m_new = jnp.maximum(m_old, jnp.max(s, axis=1, keepdims=True))
            alpha = jnp.exp(m_old - m_new)
            pr = jnp.exp(s - m_new[:, 0:1])
            l_new = alpha * l_s[...] + jnp.sum(pr, axis=1, keepdims=True)
            pv = lax.dot_general(pr.astype(jnp.bfloat16), kvbuf[slot, 1, part], NN,
                                 preferred_element_type=jnp.float32)
            acc = jnp.concatenate([alpha, alpha], axis=1) * acc_s[...] + pv
            m_s[...] = m_new
            l_s[...] = l_new
            acc_s[...] = acc

            @pl.when(c == last)
            def _():
                o = acc / jnp.concatenate([l_new, l_new], axis=1)
                keep = lax.broadcasted_iota(jnp.int32, (8, DH), 0) == 2 * p + b
                os_[2 * h] = jnp.where(keep, o, os_[2 * h])
                os_[2 * h + 1] = jnp.where(keep, pltpu.roll(o, 4, 0), os_[2 * h + 1])

        def o_cols(c0, nc):
            return jnp.concatenate([os_[j] for j in range(c0 // DH, (c0 + nc) // DH)], axis=1).astype(jnp.bfloat16)

        def o_step(g):
            w = wobuf[pl.ds(pl.multiple_of(g * 2 * GR, 2 * GR), 2 * GR), :]
            res[g] = lax.dot_general(o_cols(0, hd), w, NT, preferred_element_type=jnp.float32)

        s0 = nw + nkv - S
        i0 = s0 + lag
        tail = []
        g, s = i0, s0
        while g < total or s < total - 1:
            j = s - nw - nkv
            need = s if j < 0 else nw + nkv + max(a + n for a, n in zip(starts, phases) if a <= j) - 1
            can = s < total - 1 and (j < 0 or g >= min(need + olook, total))
            tail.append((g if g < total else -1, s if can else -1))
            g += 1
            if can:
                s += 1
                if j < 0 and s - nw - nkv < 0:
                    tail.append((-1, s))
                    s += 1

        def body(i, c):
            g = pick(i - i0, [(k, e[0]) for k, e in enumerate(tail)], i)
            s = pick(i - i0, [(k, e[1]) for k, e in enumerate(tail)], i - lag)
            t = s - nw
            j = t - nkv
            in_q = (i >= q0) & (i < q0 + nq)
            in_kv = (t >= 0) & (j < 0)
            in_o = j >= 0

            @pl.when(i == q0)
            def _():
                pltpu.make_async_copy(wqbuf, wqbuf, sem_q).wait()

            @pl.when(in_kv & (lax.rem(t, S) == 0))
            def _():
                slot = lax.rem(lax.div(t, S), NBUF)
                pltpu.make_async_copy(kvbuf.at[slot], kvbuf.at[slot], sem_kv.at[slot]).wait()

            for ph, (j0, n) in enumerate(zip(starts, phases)):
                @pl.when(j == j0)
                def _():
                    v = wobuf.at[pl.ds(j0 * 2 * GR, n * 2 * GR)]
                    pltpu.make_async_copy(v, v, sem_o.at[ph]).wait()

            issue(g)
            pl.when(i == LOOK)(prep)
            if compute:
                pl.when(in_q)(lambda: q_step(i - q0))
                pl.when(in_kv)(lambda: kv_step(t))
                pl.when(in_o)(lambda: o_step(j))
            return c

        if not compute:
            res[...] = jnp.zeros(res.shape, res.dtype)
        lax.fori_loop(0, i0 + len(tail), body, 0)

        lo = lax.broadcasted_iota(jnp.int32, (8, 128), 1) < GR

        def put(j, first, second):
            o_ref[:, pl.ds(j * 128, 128)] = jnp.where(lo, first, second)[0:nb].astype(o_ref.dtype)

        pa = [res[g] for g in range(nw - 1)]
        pb = [pltpu.roll(v, 6, 0) for v in pa]
        mid = (nw - 1) // 2
        for j in range(mid):
            put(j, pa[2 * j], pa[2 * j + 1])
        for j in range(mid - 1):
            put(mid + 1 + j, pb[2 * j + 1], pb[2 * j + 2])
        r = None
        for k in range(nlast):
            v = wobuf.at[pl.ds((nw - 1) * 2 * GR, 2 * GR), pl.ds(k * lc, lc)]
            pltpu.make_async_copy(v, v, sem_o.at[len(phases) + k]).wait()
            if compute:
                part = lax.dot_general(o_cols(k * lc, lc), v[...], NT, preferred_element_type=jnp.float32)
            else:
                part = res[0]
            r = part if r is None else r + part
        put(mid, r, pb[0])
        put(nw - 1, pb[nw - 2], pltpu.roll(r, 6, 0))

    @jax.jit
    def f(A_x, A_k_cache, A_v_cache, A_wq, A_wo, B_x, B_k_cache, B_v_cache, B_wq, B_wo):
        nb, sq, d = A_x.shape
        _, hkv, sk, dh = A_k_cache.shape
        win = min(4096, max(256, sk // 4))
        n = nb * hkv * sk
        kern = functools.partial(kernel, nb=nb, hkv=hkv, sk=sk, win=win, d=d)
        nw = d // GR
        out = pl.pallas_call(
            kern,
            in_specs=[pl.BlockSpec(memory_space=pl.ANY)] * 10,
            out_specs=pl.BlockSpec(memory_space=pltpu.VMEM),
            out_shape=jax.ShapeDtypeStruct((nb, 2 * d), A_x.dtype),
            scratch_shapes=[
                pltpu.VMEM((2, nb, d), jnp.bfloat16),
                pltpu.VMEM((nw, 2, 8, GR), jnp.float32),
                pltpu.VMEM((2, d, HQ * DH), jnp.bfloat16),
                pltpu.VMEM((2 * d, HQ * DH), jnp.bfloat16),
                pltpu.VMEM((NBUF, 2, S, R, DH), jnp.bfloat16),
                pltpu.VMEM((2, 8, HQ * DH), jnp.float32),
                pltpu.VMEM((2 * hkv, 8, DH), jnp.float32),
                pltpu.VMEM((HQ, 8, DH), jnp.float32),
                pltpu.VMEM((nw - 1, 8, 128), jnp.float32),
                pltpu.VMEM((8, 128), jnp.float32),
                pltpu.VMEM((8, 128), jnp.float32),
                pltpu.VMEM((8, DH), jnp.float32),
                pltpu.SemaphoreType.DMA(()),
                pltpu.SemaphoreType.DMA(()),
                pltpu.SemaphoreType.DMA((len(phases) + nlast,)),
                pltpu.SemaphoreType.DMA((NBUF,)),
            ],
            compiler_params=pltpu.CompilerParams(vmem_limit_bytes=64 * 1024 * 1024, disable_bounds_checks=nobc,
                                                 disable_semaphore_checks=nosc),
        )(A_x.reshape(nb, d), A_k_cache.reshape(n, dh), A_v_cache.reshape(n, dh), A_wq, A_wo.T,
          B_x.reshape(nb, d), B_k_cache.reshape(n, dh), B_v_cache.reshape(n, dh), B_wq, B_wo.T)
        return out.reshape(nb, sq, 2 * d)
    return f


if __name__ == "__main__":
    for phases, olook in (((3, 2, 1), 3), ((4, 2), 3), ((2, 2, 2), 2)):
        nw, nkv, S_, lag = 7, 160, 4, 6
        total = 2 * nw + nkv
        starts = [sum(phases[:i]) for i in range(len(phases))]
        s0 = nw + nkv - S_; i0 = s0 + lag
        tail = []
        g, s = i0, s0
        while g < total or s < total - 1:
            j = s - nw - nkv
            need = s if j < 0 else nw + nkv + max(a + n for a, n in zip(starts, phases) if a <= j) - 1
            can = s < total - 1 and (j < 0 or g >= min(need + olook, total))
            tail.append((g if g < total else -1, s if can else -1))
            g += 1
            if can:
                s += 1
                if j < 0 and s - nw - nkv < 0:
                    tail.append((-1, s))
                    s += 1
        print(phases, olook, tail)


pallas_concat_heads__gqa_block_cached__sliding_block_cached__decode_kernel = build(nlast=2)
```

```python
import functools

import jax
import jax.numpy as jnp
from jax import lax
import jax.experimental.pallas as pl
import jax.experimental.pallas.tpu as pltpu

HQ, DH = 16, 256
HD = HQ * DH
NT = (((1,), (1,)), ((), ()))
NN = (((1,), (0,)), ((), ()))

R = 1024
S = 4
SUB = 64
NBUF = 3
LAG = S + 2
GR = 64
WC = 2048
NC = HD // WC
PPG = (GR // 8) * NC
PHASES = (3, 1, 1, 1)


def _kernel(ax, ak, av, awq, awo, bx, bk, bv, bwq, bwo, o_ref,
            xbuf, xs, wqbuf, wobuf, kvbuf, ys, qs, os_, res, m_s, l_s, acc_s,
            *, nb, hkv, sk, win, d):
    nw = d // GR
    ca, cb = sk // R, win // R
    hs = nb * hkv // S
    na = nb * hkv * ca
    nkv = na + nb * hkv * cb
    total = 2 * nw + nkv
    q0 = nw + LAG - S
    qper = pl.cdiv(2 * nw, S)
    starts = [sum(PHASES[:i]) for i in range(len(PHASES))]
    assert nb == 2 and HQ == 2 * hkv and d == nw * GR and nw % 2 == 1
    assert sk % R == 0 and win % R == 0 and (nb * hkv) % S == 0 and (nw * PPG) % S == 0
    assert q0 >= nw and nw - 1 <= LAG <= (NBUF - 1) * S and sum(PHASES) == nw - 1

    def main(sem_x, sem_q, sem_kv, sem_o, sem_last):
        def wait(buf, sem):
            pltpu.make_async_copy(buf, buf, sem).wait()

        def start_wq(g):
            def body(k, carry):
                idx = g * PPG + k
                piece = lax.rem(idx, S) * (nw * PPG // S) + lax.div(idx, S)
                rows = pl.ds(pl.multiple_of(lax.div(piece, NC) * 8, 8), 8)
                cols = pl.ds(pl.multiple_of(lax.rem(piece, NC) * WC, WC), WC)
                for p, src in enumerate((awq, bwq)):
                    pltpu.make_async_copy(src.at[rows, cols], wqbuf.at[p, rows, cols],
                                          sem_q).start(priority=p)
                return carry
            lax.fori_loop(0, PPG, body, 0)

        def start_wo(blk, r, c, sem):
            cols = pl.ds(c * WC, WC)
            for p, src in enumerate((awo, bwo)):
                dst = blk * 2 * GR + (p + blk) % 2 * GR + r * 8
                pltpu.make_async_copy(src.at[pl.ds(blk * GR + r * 8, 8), cols],
                                      wobuf.at[pl.ds(dst, 8), cols], sem).start(priority=p)

        def start_kv(srcs, base, j, slot):
            for o in range(0, R // S, SUB):
                off = j * (R // S) + o
                for s in range(S):
                    rows = pl.ds(pl.multiple_of(s * hs * sk + base + off, SUB), SUB)
                    for w in range(2):
                        pltpu.make_async_copy(
                            srcs[w].at[rows],
                            kvbuf.at[slot, w, s, pl.ds(pl.multiple_of(off, SUB), SUB)],
                            sem_kv.at[slot]).start(priority=w)

        def issue(g):
            t = g - nw

            @pl.when(t < 0)
            def _():
                start_wq(g)

            @pl.when((t >= 0) & (t < na))
            def _():
                i = lax.div(t, S)
                start_kv((ak, av), i * R, lax.rem(t, S), lax.rem(i, NBUF))

            @pl.when((t >= na) & (t < nkv))
            def _():
                i = lax.div(t, S)
                u = i - na // S
                base = lax.div(u, cb) * sk + (sk - win) + lax.rem(u, cb) * R
                start_kv((bk, bv), base, lax.rem(t, S), lax.rem(i, NBUF))

            @pl.when(t >= nkv)
            def _():
                for ph, (j0, ns) in enumerate(zip(starts, PHASES)):
                    for j in range(ns):
                        @pl.when(t == nkv + j0 + j)
                        def _():
                            for k in range(j * PPG, (j + 1) * PPG):
                                piece = k // ns
                                start_wo(j0 + k % ns, piece // NC, piece % NC, sem_o.at[ph])

                @pl.when(g == total - 1)
                def _():
                    for c in range(NC):
                        for r in range(GR // 8):
                            start_wo(nw - 1, r, c, sem_last.at[c])

        def q_step(k):
            @pl.when(k == 0)
            def _():
                wait(xbuf, sem_x)
                wait(wqbuf, sem_q)
                row = lax.broadcasted_iota(jnp.int32, (8, d), 0)
                for p in range(2):
                    xv = xbuf[p].astype(jnp.float32)
                    x8 = jnp.where(row % 2 == 0, xv[0:1, :], xv[1:2, :])
                    for g in range(nw):
                        xs[g, p] = x8[:, g * GR:(g + 1) * GR]
                ys[...] = jnp.zeros(ys.shape, ys.dtype)
                os_[...] = jnp.zeros(os_.shape, os_.dtype)

            def project(u, carry):
                g, p = lax.div(u, 2), lax.rem(u, 2)
                w = wqbuf[p, pl.ds(pl.multiple_of(g * GR, GR), GR), :]
                ys[p] = ys[p] + lax.dot_general(xs[g, p].astype(jnp.bfloat16), w, NN,
                                                preferred_element_type=jnp.float32)
                return carry
            lax.fori_loop(k * qper, jnp.minimum((k + 1) * qper, 2 * nw), project, 0)

            @pl.when(k == S - 1)
            def _():
                first = lax.broadcasted_iota(jnp.int32, (8, DH), 0) < 4

                def gather(p, carry):
                    for h in range(hkv):
                        qs[p * hkv + h] = jnp.where(
                            first, ys[p, :, 2 * h * DH:(2 * h + 1) * DH],
                            ys[p, :, (2 * h + 1) * DH:(2 * h + 2) * DH])
                    return carry
                lax.fori_loop(0, 2, gather, 0)

        def kv_step(t):
            i = lax.div(t, S)
            st = lax.rem(t, S)
            slot = lax.rem(i, NBUF)
            is_b = t >= na
            u = i - na // S
            p = jnp.where(is_b, 1, 0)
            bh = st * hs + jnp.where(is_b, lax.div(u, cb), lax.div(i, ca))
            c = jnp.where(is_b, lax.rem(u, cb), lax.rem(i, ca))
            last = jnp.where(is_b, cb - 1, ca - 1)
            b = lax.div(bh, hkv)
            h = lax.rem(bh, hkv)

            @pl.when(c == 0)
            def _():
                m_s[st] = jnp.full(m_s.shape[1:], -jnp.inf, jnp.float32)
                l_s[st] = jnp.zeros(l_s.shape[1:], jnp.float32)
                acc_s[st] = jnp.zeros(acc_s.shape[1:], jnp.float32)

            q = qs[p * hkv + h].astype(jnp.bfloat16)
            s = lax.dot_general(q, kvbuf[slot, 0, st], NT,
                                preferred_element_type=jnp.float32) * (DH ** -0.5)
            m_old = m_s[st]
            m_new = jnp.maximum(m_old, jnp.max(s, axis=1, keepdims=True))
            alpha = jnp.exp(m_old - m_new)
            pr = jnp.exp(s - m_new[:, 0:1])
            l_new = alpha * l_s[st] + jnp.sum(pr, axis=1, keepdims=True)
            pv = lax.dot_general(pr.astype(jnp.bfloat16), kvbuf[slot, 1, st], NN,
                                 preferred_element_type=jnp.float32)
            acc = jnp.concatenate([alpha, alpha], axis=1) * acc_s[st] + pv
            m_s[st] = m_new
            l_s[st] = l_new
            acc_s[st] = acc

            @pl.when(c == last)
            def _():
                o = acc / jnp.concatenate([l_new, l_new], axis=1)
                keep = lax.broadcasted_iota(jnp.int32, (8, DH), 0) == 2 * p + b
                os_[2 * h] = jnp.where(keep, o, os_[2 * h])
                os_[2 * h + 1] = jnp.where(keep, pltpu.roll(o, 4, 0), os_[2 * h + 1])

        def o_step(j):
            for ph, (j0, n) in enumerate(zip(starts, PHASES)):
                @pl.when(j == j0)
                def _():
                    wait(wobuf.at[pl.ds(j0 * 2 * GR, n * 2 * GR)], sem_o.at[ph])

            lhs = jnp.concatenate([os_[k] for k in range(HQ)], axis=1).astype(jnp.bfloat16)
            w = wobuf[pl.ds(pl.multiple_of(j * 2 * GR, 2 * GR), 2 * GR), :]
            res[j] = lax.dot_general(lhs, w, NT, preferred_element_type=jnp.float32)

        def tick(g, carry):
            t = g - LAG - nw
            in_kv = (t >= 0) & (t < nkv)

            @pl.when(in_kv & (lax.rem(t, S) == 0))
            def _():
                slot = lax.rem(lax.div(t, S), NBUF)
                wait(kvbuf.at[slot], sem_kv.at[slot])

            issue(g)
            pl.when((g >= q0) & (g < q0 + S))(lambda: q_step(g - q0))
            pl.when(in_kv)(lambda: kv_step(t))
            pl.when(t >= nkv)(lambda: o_step(t - nkv))
            return carry

        pltpu.make_async_copy(ax, xbuf.at[0], sem_x).start(priority=0)
        pltpu.make_async_copy(bx, xbuf.at[1], sem_x).start(priority=1)
        lax.fori_loop(0, total - 1 + LAG, tick, 0)

        lo = lax.broadcasted_iota(jnp.int32, (8, 2 * GR), 1) < GR

        def put(j, first, second):
            tile = jnp.where(lo, first, second)[0:nb]
            o_ref[:, pl.ds(j * 2 * GR, 2 * GR)] = tile.astype(o_ref.dtype)

        pa = [res[j] for j in range(nw - 1)]
        pb = [pltpu.roll(v, 6, 0) for v in pa]
        mid = (nw - 1) // 2
        for j in range(mid):
            put(j, pa[2 * j], pa[2 * j + 1])
        for j in range(mid - 1):
            put(mid + 1 + j, pb[2 * j + 1], pb[2 * j + 2])

        def last_block(c, r):
            w = wobuf.at[pl.ds((nw - 1) * 2 * GR, 2 * GR), pl.ds(pl.multiple_of(c * WC, WC), WC)]
            heads = [os_[c * (WC // DH) + k] for k in range(WC // DH)]
            lhs = jnp.concatenate(heads, axis=1).astype(jnp.bfloat16)
            wait(w, sem_last.at[c])
            return r + lax.dot_general(lhs, w[...], NT, preferred_element_type=jnp.float32)

        r = lax.fori_loop(0, NC, last_block, jnp.zeros((8, 2 * GR), jnp.float32))
        put(mid, r, pb[0])
        put(nw - 1, pb[nw - 2], pltpu.roll(r, 6, 0))

    pl.run_scoped(
        main,
        pltpu.SemaphoreType.DMA(()),
        pltpu.SemaphoreType.DMA(()),
        pltpu.SemaphoreType.DMA((NBUF,)),
        pltpu.SemaphoreType.DMA((len(PHASES),)),
        pltpu.SemaphoreType.DMA((NC,)),
    )


@jax.jit
def pallas_concat_heads__gqa_block_cached__sliding_block_cached__decode_kernel(
    A_x: jax.Array,
    A_k_cache: jax.Array,
    A_v_cache: jax.Array,
    A_wq: jax.Array,
    A_wo: jax.Array,
    B_x: jax.Array,
    B_k_cache: jax.Array,
    B_v_cache: jax.Array,
    B_wq: jax.Array,
    B_wo: jax.Array,
):
    nb, sq, d = A_x.shape
    _, hkv, sk, dh = A_k_cache.shape
    assert sq == 1 and dh == DH and B_k_cache.shape == A_k_cache.shape
    win = min(4096, max(256, sk // 4))
    n = nb * hkv * sk
    nw = d // GR
    out = pl.pallas_call(
        functools.partial(_kernel, nb=nb, hkv=hkv, sk=sk, win=win, d=d),
        in_specs=[pl.BlockSpec(memory_space=pl.ANY)] * 10,
        out_specs=pl.BlockSpec(memory_space=pltpu.VMEM),
        out_shape=jax.ShapeDtypeStruct((nb, 2 * d), A_x.dtype),
        scratch_shapes=[
            pltpu.VMEM((2, nb, d), jnp.bfloat16),
            pltpu.VMEM((nw, 2, 8, GR), jnp.float32),
            pltpu.VMEM((2, d, HD), jnp.bfloat16),
            pltpu.VMEM((2 * d, HD), jnp.bfloat16),
            pltpu.VMEM((NBUF, 2, S, R, DH), jnp.bfloat16),
            pltpu.VMEM((2, 8, HD), jnp.float32),
            pltpu.VMEM((2 * hkv, 8, DH), jnp.float32),
            pltpu.VMEM((HQ, 8, DH), jnp.float32),
            pltpu.VMEM((nw - 1, 8, 2 * GR), jnp.float32),
            pltpu.VMEM((S, 8, 128), jnp.float32),
            pltpu.VMEM((S, 8, 128), jnp.float32),
            pltpu.VMEM((S, 8, DH), jnp.float32),
        ],
        compiler_params=pltpu.CompilerParams(vmem_limit_bytes=48 * 1024 * 1024),
    )(
        A_x.reshape(nb, d), A_k_cache.reshape(n, dh), A_v_cache.reshape(n, dh), A_wq, A_wo.T,
        B_x.reshape(nb, d), B_k_cache.reshape(n, dh), B_v_cache.reshape(n, dh), B_wq, B_wo.T,
    )
    return out.reshape(nb, sq, 2 * d)
```
